```python
import os as _os
_os.environ.setdefault("JAX_PLATFORMS", "cpu")
import jax
import jax.numpy as jnp

def _softmax(x, axis=-1):
    return jax.nn.softmax(x, axis=axis)
def _gelu(x):
    return jax.nn.gelu(x, approximate=True)
def _silu(x):
    return jax.nn.silu(x)
def _sigmoid(x):
    return jax.nn.sigmoid(x)
def _layernorm(x, axis=-1, eps=1e-5):
    m = jnp.mean(x, axis=axis, keepdims=True)
    v = jnp.var(x, axis=axis, keepdims=True)
    return (x - m) / jnp.sqrt(v + eps)
def _scatter_add(tgt, idx, src, axis=0):
    return tgt.at[idx].add(src)
def _segment_sum(src, seg, n):
    return jax.ops.segment_sum(src, seg, n)
class _Rng:
    def __init__(self, key):
        self._k = key
    def _next(self):
        self._k, sub = jax.random.split(self._k)
        return sub
    def normal(self, shape):
        return jax.random.normal(self._next(), shape, dtype=jnp.bfloat16)
    def randint(self, lo, hi, shape):
        return jax.random.randint(self._next(), shape, lo, hi, dtype=jnp.int32)
    def uniform(self, shape, lo=0.0, hi=1.0):
        return jax.random.uniform(self._next(), shape, jnp.bfloat16, lo, hi)
    def permutation(self, n):
        return jax.random.permutation(self._next(), n)


kernel_name = 'gated_mix__ssm_conv_h3__mha_block__prompt'

def setup_inputs():
    _rng = _Rng(jax.random.key(int.from_bytes(__import__("os").urandom(4), "little")))
    _w = (lambda a: (lambda t: t.astype(jnp.bfloat16) if jnp.issubdtype(t.dtype, jnp.floating) else t)(jnp.asarray(a)))
    def _A_setup():
        B, S, D = 1, 2048, 640
        ks = 4
        return {
            "q": _w((lambda *s: _rng.normal(s) * 0.05)(B, S, D)),
            "k": _w((lambda *s: _rng.normal(s) * 0.4)(B, S, D)),
            "v": _w((lambda *s: _rng.normal(s) * 0.4)(B, S, D)),
            "shift_k": _w((lambda *s: _rng.normal(s) * 0.4)(D, ks) * 0.5),
            "ssm_k": _w((lambda *s: _rng.normal(s) * 0.4)(D, S) * (1.0 / S ** 0.5)),
            "ssm_D": _w((lambda *s: _rng.normal(s) * 0.4)(D)),
        }
    _A_in = _A_setup()

    def _B_setup():
        B, S, D, H = 1, 2048, 640, 32
        return {
            "x": _w((lambda *s: _rng.normal(s) * 0.05)(B, S, D)),
            "wqkv": _w((lambda *s: _rng.normal(s) * 0.4)(D, 3 * D)),
            "wo": _w((lambda *s: _rng.normal(s) * 0.05)(D, D)),
        }
    _B_in = _B_setup()

    return {
        "A_q": _A_in["q"],
        "A_k": _A_in["k"],
        "A_v": _A_in["v"],
        "A_shift_k": _A_in["shift_k"],
        "A_ssm_k": _A_in["ssm_k"],
        "A_ssm_D": _A_in["ssm_D"],
        "B_x": _B_in["x"],
        "B_wqkv": _B_in["wqkv"],
        "B_wo": _B_in["wo"],
        "gate_w": _w((lambda *s: _rng.normal(s) * 0.05)(640) * 16.0),
    }

def reference(A_q, A_k, A_v, A_shift_k, A_ssm_k, A_ssm_D, B_x, B_wqkv, B_wo, gate_w):
    def _A_ref(q, k, v, shift_k, ssm_k, ssm_D):
        B, S, D = q.shape
        ks = shift_k.shape[-1]
        k_pad = jnp.pad(k, ((0, 0), (ks - 1, 0), (0, 0)))
        k_shift = jnp.zeros_like(k)
        for t in range(ks):
            k_shift = k_shift + k_pad[:, t:t + S, :] * shift_k[:, ks - 1 - t][None, None, :]
        kv = k_shift * v
        L = 2 * S
        kv_pad = jnp.pad(kv, ((0, 0), (0, S), (0, 0)))
        kf_pad = jnp.pad(ssm_k, ((0, 0), (0, S)))
        kv_f = (lambda x, axes=(-2,-1): jnp.fft.rfft2(x.astype(jnp.float32), axes=axes))(kv_pad[:, None, :, :], axes=(1, 2))
        kf_f = (lambda x, axes=(-2,-1): jnp.fft.rfft2(x.astype(jnp.float32), axes=axes))(kf_pad[:, None, :], axes=(1, 2))
        kf_f = (lambda x, *d: x.transpose(*d))(kf_f, 1, 2, 0)
        y_f = kv_f * kf_f[None, :, :, :]
        y = (lambda x, s, axes=(-2,-1): jnp.fft.irfft2(x, s=s, axes=axes).astype(jnp.bfloat16))(y_f, (1, L), axes=(1, 2))[:, 0, :S, :]
        y = y + kv * ssm_D[None, None, :]
        return q * y

    def _B_ref(x, wqkv, wo):
        B, S, D = x.shape
        H = 32
        Dh = D // H
        qkv = (lambda x, *d: x.transpose(*d))((x @ wqkv).reshape(B, S, 3, H, Dh), 2, 0, 3, 1, 4)
        q, k, v = qkv[0], qkv[1], qkv[2]
        scores = jnp.einsum("bhqd,bhkd->bhqk", q, k) * (Dh ** -0.5)
        p = _softmax(scores, axis=-1)
        o = jnp.einsum("bhqk,bhkd->bhqd", p, v)
        return (lambda x, *d: x.transpose(*d))(o, 0, 2, 1, 3).reshape(B, S, D) @ wo

    x = A_q
    g = _sigmoid((x * gate_w).sum(-1, keepdims=True))
    a = _A_ref(x, A_k, A_v, A_shift_k, A_ssm_k, A_ssm_D)
    b = _B_ref(x, B_wqkv, B_wo)
    return g * a + (1 - g) * b
```

```python
import math

import numpy as np
import jax
import jax.numpy as jnp
import jax.experimental.pallas as pl
import jax.experimental.pallas.tpu as pltpu

S = 2048
D = 640
H = 32
DH = 20
NT = D // 128
CB = 128
NB = S // CB
BQ = 512
NQ = S // BQ
CK = 128
RC = 512
F32 = jnp.float32
BF16 = jnp.bfloat16


def _dft_tables():
    f = np.concatenate([np.arange(0, 128, 2), np.arange(1, 128, 2)]).astype(np.float64)
    t = np.arange(128, dtype=np.float64)
    th = 2.0 * np.pi * (f[:, None] + 0.5) * t[None, :] / 256.0
    fm = np.concatenate([np.cos(th), -np.sin(th)], axis=0)
    return fm.astype(np.float32), (fm.T / 128.0).astype(np.float32)


def _nt_dot(a, b):
    return jax.lax.dot_general(a, b, (((1,), (1,)), ((), ())), preferred_element_type=F32)


def _kernel(x_ref, kin_ref, vin_ref, sk_ref, hk_ref, dv_ref, w_ref, wo_ref, gw_ref,
            fm_ref, gm_ref, out_ref,
            wt_ref, qt_ref, kk_ref, vt_ref, s_ref, m_ref, ot_ref,
            kp_ref, kv_ref, xf_ref, hf_ref, wf_ref):
    qscale = (DH ** -0.5) * math.log2(math.e)

    wt_ref[0:D, :] = w_ref[:, 0:D].T
    wt_ref[D:2 * D, :] = w_ref[:, 2 * D:3 * D].T
    lane = jax.lax.broadcasted_iota(jnp.int32, (RC, 128), 1)
    sub24 = jax.lax.broadcasted_iota(jnp.int32, (24, RC), 0)
    for r in range(S // RC):
        xr = x_ref[r * RC:(r + 1) * RC, :]
        kr = jnp.dot(xr, w_ref[:, D:2 * D], preferred_element_type=F32)
        for j in range(NT):
            kk_ref[j, r * RC:(r + 1) * RC, :] = kr[:, j * 128:(j + 1) * 128].astype(BF16)
        for j in range(NT - 1):
            kk_ref[NT + j, r * RC:(r + 1) * RC, :] = jnp.where(
                lane < 64, kr[:, (j + 1) * 128:(j + 2) * 128], kr[:, j * 128:(j + 1) * 128]).astype(BF16)
        qv = _nt_dot(wt_ref[...], xr)
        for j in range(NT):
            qt_ref[j, :, r * RC:(r + 1) * RC] = qv[j * 128:(j + 1) * 128] * qscale
        vv = qv[D:2 * D].astype(BF16).astype(F32)
        for h in range(H):
            if h % 2 == 0:
                blk = jnp.where(sub24 < DH, vv[DH * h:DH * h + 24], 1.0)
            else:
                blk = jnp.where(sub24 >= 4, vv[DH * h - 4:DH * h + DH], 1.0)
            vt_ref[h, :, r * RC:(r + 1) * RC] = blk

    kp_ref[0:8, :] = jnp.zeros((8, D), F32)
    kp_ref[8:8 + S, :] = kin_ref[...].astype(F32)
    sk = sk_ref[...].astype(F32)
    fm = fm_ref[...]
    for a in range(NB):
        base = 8 + a * CB
        ks = kp_ref[base:base + CB, :] * sk[0:1]
        for j in range(1, 4):
            ks = ks + kp_ref[base - j:base - j + CB, :] * sk[j:j + 1]
        kvb = (ks * vin_ref[a * CB:(a + 1) * CB, :].astype(F32)).astype(BF16)
        kv_ref[a * CB:(a + 1) * CB, :] = kvb
        xf_ref[a] = jnp.dot(fm, kvb, preferred_element_type=F32)
    prev = None
    for j in range(NB):
        hj = _nt_dot(fm, hk_ref[:, j * CB:(j + 1) * CB])
        if prev is None:
            hf_ref[j] = hj
        else:
            hf_ref[j, 0:64] = hj[0:64] - prev[128:192]
            hf_ref[j, 64:128] = hj[64:128] + prev[192:256]
            hf_ref[j, 128:192] = hj[128:192] + prev[0:64]
            hf_ref[j, 192:256] = hj[192:256] - prev[64:128]
        prev = hj

    def mac_body(rg, carry):
        r0 = pl.multiple_of(rg * 16, 16)
        for c in range(NB):
            accr = None
            acci = None
            for a in range(c + 1):
                xr_ = xf_ref[a, pl.ds(r0, 16), :]
                xi_ = xf_ref[a, pl.ds(128 + r0, 16), :]
                hr_ = hf_ref[c - a, pl.ds(r0, 16), :]
                hi_ = hf_ref[c - a, pl.ds(128 + r0, 16), :]
                tr = xr_ * hr_ - xi_ * hi_
                ti = xr_ * hi_ + xi_ * hr_
                accr = tr if accr is None else accr + tr
                acci = ti if acci is None else acci + ti
            wf_ref[c, pl.ds(r0, 16), :] = accr.astype(BF16)
            wf_ref[c, pl.ds(128 + r0, 16), :] = acci.astype(BF16)
        return carry

    jax.lax.fori_loop(0, 8, mac_body, 0)

    row128 = jax.lax.broadcasted_iota(jnp.int32, (128, BQ), 0)

    def load_q(h, qb):
        lo = DH * h
        ja = lo // 128
        jb = (lo + DH - 1) // 128
        cols = pl.ds(pl.multiple_of(qb * BQ, BQ), BQ)
        ra = row128 + (ja * 128 - lo)
        rb = row128 + (jb * 128 - lo)
        qa = qt_ref[ja, :, cols]
        qb_ = qt_ref[jb, :, cols]
        q = jnp.where((ra >= 0) & (ra < DH), qa, jnp.where((rb >= 0) & (rb < DH), qb_, 0.0))
        return q.astype(BF16), ja + NT * (jb - ja)

    def colmax(s):
        return jnp.max(s.reshape(CK // 8, 8, BQ), axis=0)

    def stage(hn, qbn, h, qb, odd, slot, do_pv=True):
        q, kidx = load_q(hn, qbn)
        m = None
        acc = None
        if do_pv:
            mcur = m_ref[slot][0:1]
        for c in range(S // CK):
            rows = slice(c * CK, (c + 1) * CK)
            s = jnp.dot(kk_ref[kidx, rows, :], q, preferred_element_type=F32)
            s_ref[1 - slot, rows, :] = s
            mc = colmax(s)
            m = mc if m is None else jnp.maximum(m, mc)
            if do_pv:
                p = jnp.exp2(s_ref[slot, rows, :] - mcur)
                o = jnp.dot(vt_ref[h, :, rows], p, preferred_element_type=F32)
                acc = o if acc is None else acc + o
        m_ref[1 - slot] = jnp.broadcast_to(jnp.max(m, axis=0, keepdims=True), (8, BQ))
        if do_pv:
            cols = pl.ds(pl.multiple_of(qb * BQ, BQ), BQ)
            if odd:
                r = 1.0 / acc[0:1]
                ot_ref[h // 2, DH:2 * DH, cols] = (acc * r)[4:24]
            else:
                r = 1.0 / acc[DH:DH + 1]
                ot_ref[h // 2, 0:DH, cols] = (acc * r)[0:DH]

    stage(0, 0, 0, 0, False, 1, do_pv=False)

    def attn_body(i, carry):
        hp = i // NQ
        qb = i % NQ
        h0 = 2 * hp
        stage(h0 + 1, qb, h0, qb, False, 0)
        inext = jnp.minimum(i + 1, (H // 2) * NQ - 1)
        stage(2 * (inext // NQ), inext % NQ, h0 + 1, qb, True, 1)
        return carry

    jax.lax.fori_loop(0, (H // 2) * NQ, attn_body, 0)

    gm = gm_ref[...]
    dv = dv_ref[...].astype(F32)
    gw = gw_ref[...].astype(F32)
    for r in range(S // RC):
        rows = slice(r * RC, (r + 1) * RC)
        ot = ot_ref[:, :, rows].reshape(D, RC)
        o = ot.T.astype(BF16)
        b = jnp.dot(o, wo_ref[...], preferred_element_type=F32)
        for cc in range(RC // CB):
            c = r * (RC // CB) + cc
            rws = slice(c * CB, (c + 1) * CB)
            y = jnp.dot(gm, wf_ref[c], preferred_element_type=F32)
            xr = x_ref[rws, :].astype(F32)
            g = jax.nn.sigmoid(jnp.sum(xr * gw, axis=-1, keepdims=True))
            a = xr * (y + kv_ref[rws, :].astype(F32) * dv)
            bb = b[cc * CB:(cc + 1) * CB]
            out_ref[rws, :] = (bb + g * (a - bb)).astype(out_ref.dtype)


@jax.jit
def pallas_gated_mix__ssm_conv_h3__mha_block__prompt_kernel(
    A_q: jax.Array,
    A_k: jax.Array,
    A_v: jax.Array,
    A_shift_k: jax.Array,
    A_ssm_k: jax.Array,
    A_ssm_D: jax.Array,
    B_x: jax.Array,
    B_wqkv: jax.Array,
    B_wo: jax.Array,
    gate_w: jax.Array,
):
    fm, gm = _dft_tables()
    args = (
        A_q.reshape(S, D), A_k.reshape(S, D), A_v.reshape(S, D),
        A_shift_k.T, A_ssm_k, A_ssm_D.reshape(1, D), B_wqkv, B_wo, gate_w.reshape(1, D),
        jnp.asarray(fm, BF16), jnp.asarray(gm, BF16),
    )
    out = pl.pallas_call(
        _kernel,
        out_shape=jax.ShapeDtypeStruct((S, D), BF16),
        scratch_shapes=[
            pltpu.VMEM((2 * D, D), BF16),
            pltpu.VMEM((NT, 128, S), F32),
            pltpu.VMEM((2 * NT - 1, S, 128), BF16),
            pltpu.VMEM((H, 24, S), F32),
            pltpu.VMEM((2, S, BQ), F32),
            pltpu.VMEM((2, 8, BQ), F32),
            pltpu.VMEM((H // 2, 2 * DH, S), F32),
            pltpu.VMEM((S + 8, D), F32),
            pltpu.VMEM((S, D), BF16),
            pltpu.VMEM((NB, 256, D), F32),
            pltpu.VMEM((NB, 256, D), F32),
            pltpu.VMEM((NB, 256, D), BF16),
        ],
        compiler_params=pltpu.CompilerParams(vmem_limit_bytes=120 * 2 ** 20),
    )(*args)
    return out.reshape(1, S, D)
```

```python
import math

import numpy as np
import jax
import jax.numpy as jnp
import jax.experimental.pallas as pl
import jax.experimental.pallas.tpu as pltpu

S = 2048
D = 640
H = 32
DH = 20
NP = H // 2
NT = D // 128
CB = 128
NB = S // CB
BQ = 512
NQ = S // BQ
NS = 2 * NQ
CK = 128
NC = S // CK
RC = 512
KS = 128
VGI = 6
XG = ((6, 4, 0, 6), (14, 4, 6, 14))
SHORT = tuple(x[0] + 1 for x in XG)
VG = tuple((c, VGI) for c in range(NC)) + tuple(x[:2] for x in XG)
NV = len(VG)
KEND = 63
QMIN = 2.0 ** -40
SMAX = 80.0
XS = (0, 128, 640, S)
OS = (0, 512, 1024, 1536, 1792, 1920, S)
F32 = jnp.float32
BF16 = jnp.bfloat16
U32 = jnp.uint32


def _dft_tables():
    fe = np.arange(0, 128, 2)
    f = np.concatenate([fe, 127 - fe]).astype(np.float64)
    t = np.arange(128, dtype=np.float64)
    th = 2.0 * np.pi * (f[:, None] + 0.5) * t[None, :] / 256.0
    fm = np.concatenate([np.cos(th), -np.sin(th)], axis=0)
    g = np.concatenate([np.cos(th[0:64]), -np.sin(th[0:64])], axis=0).T / 128.0
    gm = np.concatenate([g[0::2], g[1::2]], axis=0)
    return fm.astype(np.float32), gm.astype(np.float32)


def _nt_dot(a, b):
    return jax.lax.dot_general(a, b, (((1,), (1,)), ((), ())), preferred_element_type=F32)


def _pack(x):
    return pltpu.bitcast(x.astype(BF16), U32)


def _unpack(x):
    return pltpu.bitcast(x, BF16)


def _absmax8(v):
    v = jnp.max(jnp.abs(v).reshape(v.shape[0] // 8, 8, v.shape[1]), axis=0)
    m = v[:, 0:128]
    for l in range(128, v.shape[1], 128):
        m = jnp.maximum(m, v[:, l:l + 128])
    return m


def _recip(x):
    r = pl.reciprocal(x, approx=True)
    return r + r * (1.0 - x * r)


def _kernel(x_hbm, kin_hbm, vin_hbm, sk_hbm, hk_hbm, dv_hbm, w_hbm, wo_hbm, gw_hbm,
            fm_hbm, gm_hbm, out_hbm,
            x_ref, kin_ref, vin_ref, hk_ref, w_ref, wo_ref,
            fm_ref, gm_ref, out_ref, sem_in, sem_out,
            wt_ref, qt_ref, acc_ref, kk_ref, vt_ref, s_ref, pc_ref, vc_ref, mx_ref, ot_ref,
            kp_ref, kv_ref, xf_ref, hf_ref, wf_ref, zs_ref, q32_ref, k32_ref, kb_ref, qb_ref,
            sk_ref, dv_ref, gw_ref):
    qscale = (DH ** -0.5) * math.log2(math.e)

    def cp(src, dst, i):
        return pltpu.make_async_copy(src, dst, sem_in.at[i])

    c_wk = cp(w_hbm.at[:, D:2 * D], w_ref.at[:, D:2 * D], 0)
    c_x = [cp(x_hbm.at[XS[i]:XS[i + 1]], x_ref.at[XS[i]:XS[i + 1]], 1 + i) for i in range(3)]
    c_wq = cp(w_hbm.at[:, 0:D], w_ref.at[:, 0:D], 4)
    c_wv = cp(w_hbm.at[:, 2 * D:3 * D], w_ref.at[:, 2 * D:3 * D], 5)
    c_small = [cp(sk_hbm, sk_ref, 6), cp(fm_hbm, fm_ref, 7)]
    c_epi = [cp(wo_hbm, wo_ref, 8), cp(dv_hbm, dv_ref, 9), cp(gw_hbm, gw_ref, 10),
             cp(gm_hbm, gm_ref, 11)]

    def chunk(r):
        if isinstance(r, int):
            return slice(r * RC, (r + 1) * RC)
        return pl.ds(pl.multiple_of(r * RC, RC), RC)

    def c_k(r):
        return cp(kin_hbm.at[chunk(r)], kin_ref.at[chunk(r)], 12 + 3 * r)

    def c_vh(r):
        sl = chunk(r)
        return [cp(vin_hbm.at[sl], vin_ref.at[sl], 13 + 3 * r),
                cp(hk_hbm.at[:, sl], hk_ref.at[:, sl], 14 + 3 * r)]

    c_wk.start()
    for c in c_x:
        c.start()

    for i in range(NB):
        zs_ref[i] = 0
    for l in range(NT):
        kp_ref[l, 0:8, :] = jnp.zeros((8, 128), F32)
    pc_ref[...] = jnp.ones((CK, BQ), F32)
    acc_ref[...] = jnp.zeros((1, 24, BQ), F32)
    mx_ref[...] = jnp.zeros((4, 8, 128), F32)

    def pad_body(h, carry):
        q32_ref[h, :, 24:32, :] = jnp.ones((S // 128, 8, 128), F32)
        return carry

    jax.lax.fori_loop(0, H, pad_body, 0)

    def kproj(q0, q1):
        lane = jax.lax.broadcasted_iota(jnp.int32, (KS // 2, 128), 1)
        for r0 in range(q0, q1, KS):
            kr = jnp.dot(x_ref[r0:r0 + KS, :], w_ref[:, D:2 * D], preferred_element_type=F32)
            mx_ref[0] = jnp.maximum(mx_ref[0], _absmax8(kr))
            kr = _pack(kr)
            tl = [kr[:, j * 128:(j + 1) * 128] for j in range(NT)]
            for hp in range(NP):
                lo = 2 * DH * hp
                ja, jb = lo // 128, (lo + 2 * DH - 1) // 128
                src = tl[ja] if ja == jb else jnp.where(lane < 64, tl[jb], tl[ja])
                if lo % 128:
                    src = pltpu.roll(src, 128 - lo % 128, axis=1)
                kk_ref[hp, r0 // 2:(r0 + KS) // 2, :] = src
                for v, (c, i) in enumerate(VG):
                    if c == r0 // CK:
                        k32_ref[hp, v * 16:(v + 1) * 16, :] = _unpack(src[8 * i:8 * i + 8]).astype(F32)

    c_wk.wait()
    c_x[0].wait()
    c_wq.start()
    c_wv.start()
    kproj(XS[0], XS[1])
    c_x[1].wait()
    for c in c_small + [c_k(0)] + c_vh(0) + [c_k(1)]:
        c.start()
    kproj(XS[1], XS[2])
    c_x[2].wait()
    kproj(XS[2], 1536)
    c_wq.wait()
    c_wv.wait()
    c_k(0).wait()
    for c in c_vh(1) + [c_k(2)] + c_vh(2) + [c_k(3)] + c_vh(3):
        c.start()
    wt_ref[0:D, :] = w_ref[:, 0:D].T
    wt_ref[D:2 * D, :] = w_ref[:, 2 * D:3 * D].T
    for l in range(NT):
        kp_ref[l, 8:8 + RC, :] = kin_ref[0:RC, l * 128:(l + 1) * 128].astype(F32)
    kproj(1536, S)

    for c in c_small:
        c.wait()

    def qvconv_body(r, carry):
        r0 = pl.multiple_of(r * RC, RC)
        sl = pl.ds(r0, RC)
        for c in c_vh(r):
            c.wait()

        @pl.when(r + 1 < S // RC)
        def _():
            c_k(r + 1).wait()

        sn = chunk(jnp.minimum(r + 1, S // RC - 1))
        for l in range(NT):
            kp_ref[l, pl.ds(8 + RC + r0, RC), :] = kin_ref[sn, l * 128:(l + 1) * 128].astype(F32)
        sub24 = jax.lax.broadcasted_iota(jnp.int32, (24, RC), 0)
        sub32 = jax.lax.broadcasted_iota(jnp.int32, (32, RC), 0)
        qv = _nt_dot(wt_ref[...], x_ref[sl, :])
        qs = qv[0:D + 8] * qscale
        l1 = None
        for h in range(H):
            lo = DH * h
            if h % 2 == 0:
                qh = jnp.where(sub32 < DH, qs[lo:lo + 32], 0.0)
            else:
                qh = jnp.where((sub32 >= 4) & (sub32 < 24), qs[lo - 4:lo + 28], 0.0)
            qt_ref[h, :, sl] = _pack(qh)
            qr = qh[0:24].astype(BF16).astype(F32)
            qa = jnp.abs(qr)
            n1 = jnp.sum(qa, axis=0, keepdims=True)
            fill = jnp.where(sub24 < DH if h % 2 == 0 else sub24 >= 4, QMIN, 1.0)
            qc = jnp.where(qa < QMIN, fill, qr)
            for l in range(RC // 128):
                q32_ref[h, r * (RC // 128) + l, 0:24] = qc[:, l * 128:(l + 1) * 128]
            if h < 2:
                ra = qc * _recip(pltpu.roll(qc, 23, axis=0))
                for d in range(DH):
                    qb_ref[h * NQ + r, d] = jnp.broadcast_to(ra[4 * h + d:4 * h + d + 1], (8, RC))
            l1 = n1 if l1 is None else jnp.maximum(l1, n1)
        mx_ref[1] = jnp.maximum(mx_ref[1], _absmax8(jnp.broadcast_to(l1, (8, RC))))
        vv = qv[D:2 * D].astype(BF16).astype(F32)
        mx_ref[2] = jnp.maximum(mx_ref[2], _absmax8(vv))
        for h in range(H):
            if h % 2 == 0:
                blk = jnp.where(sub24 < DH, vv[DH * h:DH * h + 24], 1.0)
            else:
                blk = jnp.where(sub24 >= 4, vv[DH * h - 4:DH * h + DH], 1.0)
            vt_ref[h, :, sl] = blk
        src = _unpack(jnp.concatenate(
            [kk_ref[0, c * 64 + 8 * i:c * 64 + 8 * i + 8, :] for (c, i) in VG], axis=0)).astype(F32)
        for dd in range(DH // NQ):
            d = r * (DH // NQ) + dd
            kb_ref[0, d] = jnp.take_along_axis(src, jnp.full((NV * 16, 128), d, jnp.int32), axis=1)
        sk = sk_ref[...].astype(F32)
        fm = fm_ref[...]
        for aa in range(RC // CB):
            a = r * (RC // CB) + aa
            b0 = pl.multiple_of(r0 + aa * CB, CB)
            ks = None
            for j in range(4):
                kj = jnp.concatenate(
                    [kp_ref[l, pl.ds(8 - j + aa * CB + r0, CB), :] for l in range(NT)], axis=1)
                ks = kj * sk[0:1] if j == 0 else ks + kj * sk[j:j + 1]
            kvb = (ks * vin_ref[pl.ds(b0, CB), :].astype(F32)).astype(BF16)
            kv_ref[pl.ds(b0, CB), :] = kvb
            hfa = _nt_dot(fm, hk_ref[:, pl.ds(b0, CB)])
            xfa = jnp.dot(fm, kvb, preferred_element_type=F32)
            for u in range(32):
                hf_ref[u % 16, a, u // 16] = hfa[8 * u:8 * u + 8]
                xf_ref[u % 16, a, u // 16] = xfa[8 * u:8 * u + 8]
        return carry

    jax.lax.fori_loop(0, S // RC, qvconv_body, 0)
    for c in c_epi:
        c.start()

    zq = vt_ref[0, 0:8, 0:128]
    never = (zq != zq) & (zq > 0.0)

    steps = [(l, c, a) for l in range(NT) for c in range(0, NB, 2) for a in range(c + 2)]
    n_slots = NS * NC
    st = {}

    def mac_step(u, slot_id, sc):
        lo = len(steps) * slot_id // n_slots
        hi = len(steps) * (slot_id + 1) // n_slots
        for n, (l, c, a) in enumerate(steps[lo:hi]):
            ln = slice(l * 128, (l + 1) * 128)
            if a == 0:
                uu = u + zs_ref[c]
                st.update(u=uu, x=xf_ref[uu, 0:c + 2, :, :, ln], h=hf_ref[uu, 0:c + 2, :, :, ln])
            xr, xi = st["x"][a, 0], st["x"][a, 1]
            if sc is not None:
                j = (14 * n + 5) // (hi - lo)
                dep = sc[8 * j:8 * j + 8, 256:384]
                xr, xi = jax.lax.select(never, dep, xr), jax.lax.select(never, dep, xi)
            for cc in (c + 1, c):
                if a <= cc:
                    hr, hi_ = st["h"][cc - a, 0], st["h"][cc - a, 1]
                    tr = xr * hr - xi * hi_
                    ti = xr * hi_ + xi * hr
                    st[cc] = (tr, ti) if a == 0 else (st[cc][0] + tr, st[cc][1] + ti)
            if a >= c:
                wf_ref[st["u"], a, 0, :, ln] = st[a][0]
                wf_ref[st["u"], a, 1, :, ln] = st[a][1]

    def head_of(t):
        return t // NQ, t % NQ

    def load_q(h, par, cols):
        q = _unpack(qt_ref[h, :, cols])
        if par:
            q = jnp.concatenate([jnp.zeros((16, BQ), BF16), q], axis=0)
        return q

    def store_o(pp, par, cols, acc):
        if par:
            ot_ref[pp, DH:2 * DH, cols] = (acc * (1.0 / acc[0:1]))[4:24]
        else:
            ot_ref[pp, 0:DH, cols] = (acc * (1.0 / acc[DH:DH + 1]))[0:DH]

    def kb_gen(hp, par, d, dep):
        idx = jnp.full((8, 128), par * DH + d, jnp.int32)
        if dep is not None:
            idx = jax.lax.select(never, pltpu.bitcast(dep, jnp.int32), idx)
        idx = jnp.concatenate([idx] * (2 * NV), axis=0)
        kb_ref[par, d] = jnp.take_along_axis(k32_ref[hp], idx, axis=1)

    def qb_gen(hp, t, e, dep):
        par, qi = head_of(t)
        rt, l = e % 3, (e // 3) * 128
        tile = qi * (BQ // 128) + e // 3
        wn = jax.lax.select(never, dep, q32_ref[2 * hp + par, tile, rt * 8 + 1:rt * 8 + 9, :])
        w = q32_ref[2 * hp + par, tile, rt * 8:rt * 8 + 8, :] * _recip(wn)
        for r in range(8):
            d = rt * 8 + r - 4 * par
            if 0 <= d < DH:
                qb_ref[t, d, :, l:l + 128] = jnp.broadcast_to(w[r:r + 1], (8, 128))

    order = [(c, i) for c in range(NC) for i in reversed(range(8)) if (c, i) not in VG]
    cuts = [0]
    for c in range(NC):
        cuts.append(cuts[-1] + (6 if c in SHORT else 7))

    def pv(hp, g, p):
        t, c = g // NC, g % NC
        par, qi = head_of(t % NS)
        if g >= 0:
            pp, hv = hp, 2 * hp + par
        elif isinstance(hp, int):
            pp, hv = hp - 1, 2 * hp - 1
        else:
            pp, hv = jnp.where(hp == 0, NP, hp - 1), jnp.maximum(2 * hp - 1, 0)
        o = jnp.dot(vt_ref[hv, :, c * CK:(c + 1) * CK], p, preferred_element_type=F32)
        if c > 0:
            o = o + acc_ref[zs_ref[c]]
        if c == NC - 1:
            store_o(pp, par, slice(qi * BQ, (qi + 1) * BQ), o)
        else:
            acc_ref[0] = o

    def vpu_steps(t, v, d0, d1, acc, pins):
        kbs = kb_ref[head_of(t)[0], d0:d1, v * 16:(v + 1) * 16, :]
        qbs = qb_ref[t, d0:d1]
        for d in range(d0, d1):
            kb, qb = kbs[d - d0], qbs[d - d0]
            if d in pins:
                kb = jnp.concatenate([jax.lax.select(never, dep, kb[i:i + 8])
                                      for dep, i in zip(pins[d], (0, 8))], axis=0)
            kb = jnp.concatenate([kb] * (BQ // 128), axis=1)
            acc = (kb if d == 0 else acc + kb) * jnp.concatenate([qb, qb], axis=0)
        return acc

    def vpu_block(t, v, sp):
        pins = {}
        if sp is not None:
            for d in (0, 1, 6, 11, 16):
                j = (sp.shape[0] // 8) * d // DH
                pins[d] = [sp[8 * j:8 * j + 8, l:l + 128] for l in (0, 256)]
        return jnp.exp2(vpu_steps(t, v, 0, DH, None, pins))

    def fast_body(hp, carry):
        hn = jnp.minimum(hp + 1, NP - 1)
        sprev = None
        pprev = pc_ref[...]
        pg = {}
        xacc = None
        for g in range(NS * NC):
            t, c = g // NC, g % NC
            par, qi = head_of(t)
            q = load_q(2 * hp + par + zs_ref[c], par, slice(qi * BQ, (qi + 1) * BQ))
            gq = qi * NC + c
            gens = range(DH * min(gq, KEND) // KEND, DH * min(gq + 1, KEND) // KEND)
            if not par:
                for d in gens:
                    kb_gen(hp, 1, d, None)
            grp = order[cuts[c]:cuts[c + 1]]
            kt = {cc: kk_ref[hp, cc * 64:(cc + 1) * 64, :] for cc in sorted({cc for cc, _ in grp})}
            kc = _unpack(jnp.concatenate([kt[cc][i * 8:i * 8 + 8] for (cc, i) in grp], axis=0))
            s = jnp.dot(kc[:, 0:q.shape[0]], q, preferred_element_type=F32)
            ex = jnp.exp2(s)
            for n, ci in enumerate(grp):
                pg[ci] = ex[16 * n:16 * n + 16]
            pg[(c, VGI)] = vc_ref[...] if g == 0 else vpu_block(t, c, sprev)
            for xi, (xc, xg, s0, s1) in enumerate(XG):
                if s0 <= c < s1:
                    d0, d1 = DH * (c - s0) // (s1 - s0), DH * (c + 1 - s0) // (s1 - s0)
                    last = s[s.shape[0] - 8:, 256:384]
                    xacc = vpu_steps(t, NC + xi, d0, d1, xacc, {d0: [last, last]})
                    if d1 == DH:
                        pg[(xc, xg)] = jnp.exp2(xacc)
            if par:
                for d in gens:
                    kb_gen(hn, 0, d, s[0:8, 0:128])
            if c >= 4:
                qb_gen(hn if t > 0 else hp, (t - 1) % NS, c - 4, s[88:96, 0:128])
            pv(hp, g - 1, pprev)
            pprev = jnp.concatenate([pg.pop((c, i)) for i in range(8)], axis=0)
            mac_step(hp, g, s)
            sprev = s
        pc_ref[...] = pprev
        vc_ref[...] = vpu_block(0, 0, sprev)
        return carry

    def fast_path():
        jax.lax.fori_loop(0, NP, fast_body, 0)
        pv(NP, -1, pc_ref[...])

    def safe_body(i, carry):
        hp = i // NQ
        cols = pl.ds(pl.multiple_of((i % NQ) * BQ, BQ), BQ)
        for par in range(2):
            q = load_q(2 * hp + par, par, cols)

            def qk(c, m):
                kc = _unpack(kk_ref[hp, pl.ds(pl.multiple_of(c * 64, 64), 64), :])
                s = jnp.dot(kc[:, 0:q.shape[0]], q, preferred_element_type=F32)
                s_ref[pl.ds(pl.multiple_of(c * CK, CK), CK), :] = s
                return jnp.maximum(m, jnp.max(s.reshape(CK // 8, 8, BQ), axis=0))

            m = jax.lax.fori_loop(0, NC, qk, jnp.full((8, BQ), -jnp.inf, F32), unroll=4)
            m = jnp.max(m, axis=0, keepdims=True)

            def pvs(c, acc):
                rows = pl.ds(pl.multiple_of(c * CK, CK), CK)
                p = jnp.exp2(s_ref[rows, :] - m)
                return jnp.dot(vt_ref[2 * hp + par, :, rows], p, preferred_element_type=F32) + acc

            store_o(hp, par, cols, jax.lax.fori_loop(0, NC, pvs, jnp.zeros((24, BQ), F32), unroll=4))
        return carry

    def mac_body(u, carry):
        for g in range(n_slots):
            mac_step(u, g, None)
        return carry

    def safe_path():
        jax.lax.fori_loop(0, NP * NQ, safe_body, 0)
        jax.lax.fori_loop(0, NP, mac_body, 0)

    vc_ref[...] = vpu_block(0, 0, None)
    kmax = jnp.max(mx_ref[0])
    vmax = jnp.max(mx_ref[2])
    ok = ((kmax * jnp.max(mx_ref[1]) * 1.02 <= SMAX) & (vmax >= 2.0 ** -20) & (vmax <= 2.0 ** 30)
          & (kmax >= 2.0 ** -60) & (kmax <= 2.0 ** 10))
    jax.lax.cond(ok, fast_path, safe_path)

    for c in c_epi:
        c.wait()

    gm = gm_ref[...]
    dv = dv_ref[...].reshape(1, D).astype(F32)
    gw = gw_ref[...].reshape(1, D).astype(F32)
    outs = []

    def inv_dft(c):
        w = jnp.concatenate([wf_ref[u % 16, c, u // 16] for u in range(32)], axis=0)
        r1, r2, i1, i2 = w[0:64], w[64:128], w[128:192], w[192:256]
        if c > 0:
            wp = jnp.concatenate([wf_ref[u % 16, c - 1, u // 16] for u in range(32)], axis=0)
            r1, r2, i1, i2 = r1 - wp[128:192], r2 + wp[192:256], i1 + wp[0:64], i2 - wp[64:128]
        u = jnp.concatenate([r1 + r2, i1 - i2], axis=0).astype(BF16)
        v = jnp.concatenate([r1 - r2, i1 + i2], axis=0).astype(BF16)
        ye = jnp.dot(gm[0:64], u, preferred_element_type=F32)
        yo = jnp.dot(gm[64:128], v, preferred_element_type=F32)
        for l in range(NT):
            kp_ref.at[l][pl.ds(c * CB, 64, stride=2), :] = ye[:, l * 128:(l + 1) * 128]
            kp_ref.at[l][pl.ds(c * CB + 1, 64, stride=2), :] = yo[:, l * 128:(l + 1) * 128]

    inv_dft(0)
    for c in range(NB):
        rws = slice(c * CB, (c + 1) * CB)
        if c + 1 < NB:
            inv_dft(c + 1)
        o = ot_ref[0:NP, :, rws].reshape(D, CB).T.astype(BF16)
        bb = jnp.dot(o, wo_ref[...], preferred_element_type=F32)
        y = jnp.concatenate([kp_ref[l, rws, :] for l in range(NT)], axis=1)
        xr = x_ref[rws, :].astype(F32)
        g = jax.nn.sigmoid(jnp.sum(xr * gw, axis=-1, keepdims=True))
        a = xr * (y + kv_ref[rws, :].astype(F32) * dv)
        out_ref[rws, :] = (bb + g * (a - bb)).astype(out_ref.dtype)
        if (c + 1) * CB in OS:
            i = OS.index((c + 1) * CB)
            rows = slice(OS[i - 1], OS[i])
            oc = pltpu.make_async_copy(out_ref.at[rows], out_hbm.at[rows], sem_out.at[i - 1])
            oc.start()
            outs.append(oc)
    for oc in outs:
        oc.wait()


@jax.jit
def pallas_gated_mix__ssm_conv_h3__mha_block__prompt_kernel(
    A_q: jax.Array,
    A_k: jax.Array,
    A_v: jax.Array,
    A_shift_k: jax.Array,
    A_ssm_k: jax.Array,
    A_ssm_D: jax.Array,
    B_x: jax.Array,
    B_wqkv: jax.Array,
    B_wo: jax.Array,
    gate_w: jax.Array,
):
    fm, gm = _dft_tables()
    args = (
        A_q.reshape(S, D), A_k.reshape(S, D), A_v.reshape(S, D),
        A_shift_k.T, A_ssm_k, A_ssm_D, B_wqkv, B_wo, gate_w,
        jnp.asarray(fm, BF16), jnp.asarray(gm, BF16),
    )
    out = pl.pallas_call(
        _kernel,
        out_shape=jax.ShapeDtypeStruct((S, D), BF16),
        in_specs=[pl.BlockSpec(memory_space=pl.ANY)] * len(args),
        out_specs=pl.BlockSpec(memory_space=pl.ANY),
        scratch_shapes=[pltpu.VMEM(args[i].shape, BF16) for i in (0, 1, 2, 4, 6, 7, 9, 10)] + [
            pltpu.VMEM((S, D), BF16),
            pltpu.SemaphoreType.DMA((12 + 3 * (S // RC),)),
            pltpu.SemaphoreType.DMA((len(OS) - 1,)),
            pltpu.VMEM((2 * D, D), BF16),
            pltpu.VMEM((H, 16, S), U32),
            pltpu.VMEM((1, 24, BQ), F32),
            pltpu.VMEM((NP, S // 2, 128), U32),
            pltpu.VMEM((H, 24, S), F32),
            pltpu.VMEM((S, BQ), F32),
            pltpu.VMEM((CK, BQ), F32),
            pltpu.VMEM((16, BQ), F32),
            pltpu.VMEM((4, 8, 128), F32),
            pltpu.VMEM((NP + 1, 2 * DH, S), F32),
            pltpu.VMEM((NT, S + RC + 32, 128), F32),
            pltpu.VMEM((S, D), BF16),
            pltpu.VMEM((16, NB, 2, 8, D), F32),
            pltpu.VMEM((16, NB, 2, 8, D), F32),
            pltpu.VMEM((16, NB, 2, 8, D), F32),
            pltpu.SMEM((NB,), jnp.int32),
            pltpu.VMEM((H, S // 128, 32, 128), F32),
            pltpu.VMEM((NP, NV * 16, 128), F32),
            pltpu.VMEM((2, DH, NV * 16, 128), F32),
            pltpu.VMEM((NS, DH, 8, BQ), F32),
        ] + [pltpu.VMEM(args[i].shape, BF16) for i in (3, 5, 8)],
        compiler_params=pltpu.CompilerParams(vmem_limit_bytes=124 * 2 ** 20),
    )(*args)
    return out.reshape(1, S, D)
```
